```python
import jax
import jax.numpy as jnp

def _softmax(x, axis=-1):
    return jax.nn.softmax(x, axis=axis)
def _gelu(x):
    return jax.nn.gelu(x, approximate=True)
def _silu(x):
    return jax.nn.silu(x)
def _sigmoid(x):
    return jax.nn.sigmoid(x)
def _layernorm(x, axis=-1, eps=1e-5):
    m = jnp.mean(x, axis=axis, keepdims=True)
    v = jnp.var(x, axis=axis, keepdims=True)
    return (x - m) / jnp.sqrt(v + eps)
def _scatter_add(tgt, idx, src, axis=0):
    return tgt.at[idx].add(src)
def _segment_sum(src, seg, n):
    return jax.ops.segment_sum(src, seg, n)
class _Rng:
    def __init__(self, key):
        self._k = key
    def _next(self):
        self._k, sub = jax.random.split(self._k)
        return sub
    def normal(self, shape):
        return jax.random.normal(self._next(), shape, dtype=jnp.bfloat16)
    def randint(self, lo, hi, shape):
        return jax.random.randint(self._next(), shape, lo, hi, dtype=jnp.int32)
    def uniform(self, shape, lo=0.0, hi=1.0):
        return jax.random.uniform(self._next(), shape, jnp.bfloat16, lo, hi)
    def permutation(self, n):
        return jax.random.permutation(self._next(), n)


kernel_name = 'interleave_layers__sliding_block_cached__dense_activation_gelu__decode'

def setup_inputs():
    _rng = _Rng(jax.random.key(int.from_bytes(__import__("os").urandom(4), "little")))
    _w = (lambda a: (lambda t: t.astype(jnp.bfloat16) if jnp.issubdtype(t.dtype, jnp.floating) else t)(jnp.asarray(a)))
    def _A_setup():
        B, Sq, D = 1, 1, 640
        Hq, Hkv, Sk, Dh = 32, 32, 32768, 192
        assert Hq % Hkv == 0, (Hq, Hkv)
        return {
            "x": _w((lambda *s: _rng.normal(s) * 0.05)(B, Sq, D)),
            "k_cache": _w((lambda *s: _rng.normal(s) * 0.05)(B, Hkv, Sk, Dh)),
            "v_cache": _w((lambda *s: _rng.normal(s) * 0.05)(B, Hkv, Sk, Dh)),
            "wq": _w((lambda *s: _rng.normal(s) * 0.05)(D, Hq * Dh) * (D ** -0.5)),
            "wo": _w((lambda *s: _rng.normal(s) * 0.05)(Hq * Dh, D) * ((Hq * Dh) ** -0.5)),
        }
    _A_in = _A_setup()

    def _B_setup():
        B, S, D, F = 1, 1, 640, 1536
        return {
            "x": _w((lambda *s: _rng.normal(s) * 0.05)(B, S, D)),
            "w1": _w((lambda *s: _rng.normal(s) * 0.05)(D, F) * (D ** -0.5)),
            "b1": _w((lambda *s: _rng.normal(s) * 0.05)(F) * 0.01),
            "w2": _w((lambda *s: _rng.normal(s) * 0.05)(F, D) * (F ** -0.5)),
            "b2": _w((lambda *s: _rng.normal(s) * 0.05)(D) * 0.01),
        }
    _B_in = _B_setup()

    return {
        "A_x": _A_in["x"],
        "A_k_cache": _A_in["k_cache"],
        "A_v_cache": _A_in["v_cache"],
        "A_wq": _A_in["wq"],
        "A_wo": _A_in["wo"],
        "B_x": _B_in["x"],
        "B_w1": _B_in["w1"],
        "B_b1": _B_in["b1"],
        "B_w2": _B_in["w2"],
        "B_b2": _B_in["b2"],
    }

def reference(A_x, A_k_cache, A_v_cache, A_wq, A_wo, B_x, B_w1, B_b1, B_w2, B_b2):
    def _A_ref(x, k_cache, v_cache, wq, wo):
        B, Sq, D = x.shape
        Hq, Dh = 32, 192
        Hkv, Sk = k_cache.shape[1], k_cache.shape[2]
        W = min(4096, max(256, Sk // 4))
        rep = Hq // Hkv
        q = (lambda x, *d: x.transpose(*d))((x @ wq).reshape(B, Sq, Hq, Dh), 0, 2, 1, 3)
        k = jnp.repeat(k_cache[:, :, Sk - W:, :], rep, axis=1)
        v = jnp.repeat(v_cache[:, :, Sk - W:, :], rep, axis=1)
        scores = jnp.einsum("bhqd,bhkd->bhqk", q, k) * (Dh ** -0.5)
        p = _softmax(scores, axis=-1)
        o = jnp.einsum("bhqk,bhkd->bhqd", p, v)
        return (lambda x, *d: x.transpose(*d))(o, 0, 2, 1, 3).reshape(B, Sq, Hq * Dh) @ wo

    def _B_ref(x, w1, b1, w2, b2):
        h = jnp.einsum("bsd,df->bsf", x, w1) + b1
        h = _gelu(h)
        return jnp.einsum("bsf,fd->bsd", h, w2) + b2

    x = A_x
    x = x + _A_ref(_layernorm(x, axis=-1), A_k_cache, A_v_cache, A_wq, A_wo)
    x = x + _B_ref(_layernorm(x, axis=-1), B_w1, B_b1, B_w2, B_b2)
    x = x + _A_ref(_layernorm(x, axis=-1), A_k_cache, A_v_cache, A_wq, A_wo)
    x = x + _B_ref(_layernorm(x, axis=-1), B_w1, B_b1, B_w2, B_b2)
    return x
```

```python
import jax
import jax.numpy as jnp
from jax import lax
import jax.experimental.pallas as pl
import jax.experimental.pallas.tpu as pltpu

H, DH, D, F = 32, 192, 640, 1536
SK, W = 32768, 4096
G = 8
NG = H // G
GR = G * DH
RB = GR // 16
NT = W // 128
EPS = 1e-5
BF, F32 = jnp.bfloat16, jnp.float32


def _tiles_view(a):
    r, c = a.shape
    return a.reshape(r // 16, 2, 8, c // 128, 128).transpose(0, 1, 3, 2, 4)


def _ld(buf, rows, col):
    w = buf.bitcast(jnp.uint32)[rows, col]
    return pltpu.bitcast(w.reshape(w.shape[0] * 8, 128), BF)


def _dot(a, b):
    return jnp.dot(a, b, preferred_element_type=F32)


def _layernorm(x):
    m = jnp.sum(x, axis=-1, keepdims=True) * (1.0 / D)
    c = x - m
    v = jnp.sum(c * c, axis=-1, keepdims=True) * (1.0 / D)
    return c / jnp.sqrt(v + EPS)


def _kernel(x_ref, b1_ref, b2_ref, k_hbm, v_hbm, wq_hbm, wo_hbm, w1_hbm, w2_hbm,
            o_ref, kb, vb, wqb, wob, w1b, w2b, q_ref, s_ref, l_ref, a_ref, sems):
    def copies(src, dst, r0, nr, c0, sem):
        nc = dst.shape[1]
        return [pltpu.make_async_copy(
            src.at[pl.ds(r0, nr), a, pl.ds(c0, nc)],
            dst.at[pl.ds(r0, nr), :, pl.ds(8 * a, 8), :],
            sems.at[sem, a]) for a in range(2)]

    c0 = (SK - W) // 128
    k_cp = lambda g: copies(k_hbm, kb, g * RB, RB, c0, 1 + g)
    v_cp = lambda g: copies(v_hbm, vb, g * RB, RB, c0, 1 + NG + g)
    wq_cp = copies(wq_hbm, wqb, 0, D // 16, 0, 0)
    wo_cp = copies(wo_hbm, wob, 0, H * DH // 16, 0, 1 + 2 * NG)
    w1_cp = copies(w1_hbm, w1b, 0, D // 16, 0, 2 + 2 * NG)
    w2_cp = copies(w2_hbm, w2b, 0, F // 16, 0, 3 + 2 * NG)
    stream = ([wq_cp] + [k_cp(g) for g in range(NG)] + [v_cp(g) for g in range(NG)]
              + [wo_cp, w1_cp, w2_cp])
    for cps in stream:
        for c in cps:
            c.start()

    def wait_first(first, cps):
        @pl.when(first)
        def _():
            for c in cps:
                c.wait()

    col = lax.broadcasted_iota(jnp.int32, (G, GR), 1)
    row = lax.broadcasted_iota(jnp.int32, (G, GR), 0)
    diag = (col >= row * DH) & (col < (row + 1) * DH)

    def layer(it, x):
        first = it == 0

        xn = _layernorm(x).astype(BF)
        wait_first(first, wq_cp)
        for c in range(H * DH // 128):
            g, j = divmod(c, GR // 128)
            q_ref[g, :, j * 128:(j + 1) * 128] = _dot(xn, _ld(wqb, slice(None), c))

        def scores(g, carry):
            wait_first(first, k_cp(g))
            qbd = jnp.where(diag, q_ref[g], 0.0).astype(BF)
            for t in range(NT):
                s_ref[g, :, t * 128:(t + 1) * 128] = _dot(qbd, _ld(kb, pl.ds(g * RB, RB), t))
            return carry
        lax.fori_loop(0, NG, scores, 0)

        for g in range(NG):
            s = s_ref[g] * (DH ** -0.5)
            e = jnp.exp(s - jnp.max(s, axis=-1, keepdims=True))
            s_ref[g] = e
            l_ref[g] = jnp.broadcast_to(jnp.sum(e, axis=-1, keepdims=True), (G, 128))

        def pv(g, carry):
            @pl.when(first)
            def _():
                for c in v_cp(g):
                    c.wait()

                def xpose(c, carry):
                    rows = pl.ds(g * RB + 8 * c, 8)
                    for t in range(NT):
                        tt = pltpu.bitcast(_ld(vb, rows, t).T, jnp.uint32)
                        vb.bitcast(jnp.uint32)[rows, t] = tt.reshape(8, 8, 128)
                    return carry
                lax.fori_loop(0, GR // 128, xpose, 0)

            p = s_ref[g].astype(BF)
            inv = 1.0 / l_ref[g]
            for c in range(GR // 128):
                rows = pl.ds(g * RB + 8 * c, 8)
                vt = jnp.concatenate([_ld(vb, rows, t) for t in range(NT)], axis=0)
                sl = slice(c * 128, (c + 1) * 128)
                a_ref[g, :, sl] = jnp.where(diag[:, sl], _dot(p, vt) * inv, 0.0)
            return carry
        lax.fori_loop(0, NG, pv, 0)

        wait_first(first, wo_cp)
        a = jnp.concatenate([a_ref[g].astype(BF) for g in range(NG)], axis=1)
        y = jnp.concatenate([_dot(a, _ld(wob, slice(None), c)) for c in range(D // 128)], axis=1)
        x = x + jnp.sum(y, axis=0, keepdims=True)

        xn = _layernorm(x).astype(BF)
        wait_first(first, w1_cp)
        h = jnp.concatenate([_dot(xn, _ld(w1b, slice(None), c)) for c in range(F // 128)], axis=1)
        h = jax.nn.gelu(h + b1_ref[...].astype(F32), approximate=True).astype(BF)
        wait_first(first, w2_cp)
        y = jnp.concatenate([_dot(h, _ld(w2b, slice(None), c)) for c in range(D // 128)], axis=1)
        return x + (y + b2_ref[...].astype(F32))

    x0 = jnp.broadcast_to(x_ref[0].astype(F32), (8, D))
    x = lax.fori_loop(0, 2, layer, x0)
    o_ref[0] = x[0:1].astype(o_ref.dtype)


@jax.jit
def pallas_interleave_layers__sliding_block_cached__dense_activation_gelu__decode_kernel(
    A_x: jax.Array,
    A_k_cache: jax.Array,
    A_v_cache: jax.Array,
    A_wq: jax.Array,
    A_wo: jax.Array,
    B_x: jax.Array,
    B_w1: jax.Array,
    B_b1: jax.Array,
    B_w2: jax.Array,
    B_b2: jax.Array,
):
    del B_x
    kt = _tiles_view(jnp.swapaxes(A_k_cache, 2, 3).reshape(H * DH, SK))
    vt = _tiles_view(jnp.swapaxes(A_v_cache, 2, 3).reshape(H * DH, SK))
    vmem = pl.BlockSpec(memory_space=pltpu.VMEM)
    hbm = pl.BlockSpec(memory_space=pl.ANY)
    return pl.pallas_call(
        _kernel,
        out_shape=jax.ShapeDtypeStruct(A_x.shape, A_x.dtype),
        in_specs=[vmem] * 3 + [hbm] * 6,
        out_specs=vmem,
        scratch_shapes=[
            pltpu.VMEM((H * DH // 16, NT, 16, 128), BF),
            pltpu.VMEM((H * DH // 16, NT, 16, 128), BF),
            pltpu.VMEM((D // 16, H * DH // 128, 16, 128), BF),
            pltpu.VMEM((H * DH // 16, D // 128, 16, 128), BF),
            pltpu.VMEM((D // 16, F // 128, 16, 128), BF),
            pltpu.VMEM((F // 16, D // 128, 16, 128), BF),
            pltpu.VMEM((NG, G, GR), F32),
            pltpu.VMEM((NG, G, W), F32),
            pltpu.VMEM((NG, G, 128), F32),
            pltpu.VMEM((NG, G, GR), F32),
            pltpu.SemaphoreType.DMA((4 + 2 * NG, 2)),
        ],
        compiler_params=pltpu.CompilerParams(vmem_limit_bytes=126 * 1024 * 1024),
    )(A_x, B_b1.reshape(1, F), B_b2.reshape(1, D), kt, vt,
      _tiles_view(A_wq), _tiles_view(A_wo), _tiles_view(B_w1), _tiles_view(B_w2))
```

```python
import jax
import jax.numpy as jnp
from jax import lax
import jax.experimental.pallas as pl
import jax.experimental.pallas.tpu as pltpu

H, DH, D, F = 32, 192, 640, 1536
SK, W = 32768, 4096
G = 8
NG = H // G
GR = G * DH
RB = GR // 16
NT = W // 128
MC = 8
MB = MC * 8
VB = RB - MB
TC = 4
P = 2
LAG = 4
EPS = 1e-5
BF, F32 = jnp.bfloat16, jnp.float32


def _tiles_view(a):
    r, c = a.shape
    return a.reshape(r // 16, 2, 8, c // 128, 128).transpose(0, 1, 3, 2, 4)


def _ld(buf, rows, col, zero=None):
    w = buf.bitcast(jnp.uint32)[rows, col]
    w = w.reshape(w.shape[0] * 8, 128)
    if zero is not None:
        w = jnp.concatenate([w[:-8], w[-8:] | zero], axis=0)
    return pltpu.bitcast(w, BF)


def _tie(zero, acc):
    return zero & pltpu.bitcast(acc, jnp.uint32)


def _unpack(w):
    return pltpu.bitcast(w << 16, F32), pltpu.bitcast(w & jnp.uint32(0xFFFF0000), F32)


def _dot(a, b):
    return jnp.dot(a, b, preferred_element_type=F32)


def _layernorm(x):
    m = jnp.sum(x, axis=-1, keepdims=True) * (1.0 / D)
    c = x - m
    v = jnp.sum(c * c, axis=-1, keepdims=True) * (1.0 / D)
    return c / jnp.sqrt(v + EPS)


def _kernel(x_hbm, b1_hbm, b2_hbm, k_hbm, v_hbm, wq_hbm, wo_hbm, w1_hbm, w2_hbm,
            o_ref, kb, vb, wqb, wob, w1b, w2b, q_ref, s_ref, l_ref, a_ref,
            qm_ref, acc_ref, x_ref, b1_ref, b2_ref, sems, small_sems):
    def copies(src, dst, r0, nr, c0, sem):
        nc = src.shape[2] - c0
        return [pltpu.make_async_copy(
            src.at[pl.ds(r0, nr), a, pl.ds(c0, nc)],
            dst.at[pl.ds(r0, nr), pl.ds(0, nc), pl.ds(8 * a, 8), :],
            sems.at[sem, a]) for a in range(2)]

    c0 = (SK - W) // 128
    k_cp = lambda g: copies(k_hbm, kb, g * RB, RB, c0, 1 + g)
    v_cp = lambda g: copies(v_hbm, vb, g * RB, RB, c0, 1 + NG + g)
    wq_cp = copies(wq_hbm, wqb, 0, D // 16, 0, 0)
    wo_cp = copies(wo_hbm, wob, 0, H * DH // 16, 0, 1 + 2 * NG)
    w1_cp = copies(w1_hbm, w1b, 0, D // 16, 0, 2 + 2 * NG)
    w2_cp = copies(w2_hbm, w2b, 0, F // 16, 0, 3 + 2 * NG)
    small = [pltpu.make_async_copy(s, d, small_sems.at[i]) for i, (s, d) in enumerate(
        [(x_hbm, x_ref), (b1_hbm, b1_ref), (b2_hbm, b2_ref)])]
    stream = ([wq_cp, small] + [k_cp(g) for g in range(NG)] + [v_cp(g) for g in range(NG)]
              + [wo_cp, w1_cp, w2_cp])
    for cps in stream:
        for c in cps:
            c.start()

    def wait_first(first, cps):
        @pl.when(first)
        def _():
            for c in cps:
                c.wait()

    col = lax.broadcasted_iota(jnp.int32, (G, GR), 1)
    row = lax.broadcasted_iota(jnp.int32, (G, GR), 0)
    diag = (col >= row * DH) & (col < (row + 1) * DH)
    sub = lax.broadcasted_iota(jnp.int32, (8, 128), 0)
    odd = (sub & 1) != 0
    bit1 = (sub & 2) != 0

    def layer(it, x):
        first = it == 0
        zero = jnp.full((8, 128), it >> 1, jnp.int32).astype(jnp.uint32)

        xn = _layernorm(x).astype(BF)
        wait_first(first, wq_cp)
        nj = GR // 128
        ties = []
        for g in range(NG):
            for j in range(MC, nj):
                q = _dot(xn, _ld(wqb, slice(None), g * nj + j))
                qc = jnp.broadcast_to(q[0:1], (128, 128)).astype(BF).T
                for e, w in enumerate(_unpack(pltpu.bitcast(qc, jnp.uint32))):
                    qm_ref[g, e, (j - MC) * 64:(j - MC + 1) * 64] = w
                ties.append(_tie(zero, w[56:64]))
        ties = [None] * 4 + ties
        for g in range(NG):
            for j in range(MC):
                z = ties.pop(0) if ties else None
                w = jnp.concatenate([_ld(wqb, pl.ds(8 * r, 8), g * nj + j, z) for r in range(D // 128)])
                sl = slice(j * 128, (j + 1) * 128)
                q_ref[g, :, sl] = jnp.where(diag[:, sl], _dot(xn, w), 0.0)

        wait_first(first, [c for g in range(NG) for c in k_cp(g)])
        zs = [zero] * LAG
        for g in range(NG):
            qbd = q_ref[g].astype(BF)
            ku = kb.bitcast(jnp.uint32)
            for t0 in range(0, NT, TC):
                ts = range(t0, t0 + TC)
                acc = [{} for _ in ts]
                kt = []
                for i in range(MB, RB):
                    qlo = qm_ref[g, 0, (i - MB) * 8:(i - MB + 1) * 8]
                    qhi = qm_ref[g, 1, (i - MB) * 8:(i - MB + 1) * 8]
                    h = i // (DH // 16)
                    for n, t in enumerate(ts):
                        lo, hi = _unpack(ku[g * RB + i, t])
                        term = lo * qlo + hi * qhi
                        acc[n][h] = acc[n][h] + term if h in acc[n] else term
                    zs.append(_tie(zs[-1], acc[i % TC][h]))
                    n, c = divmod(i - MB, MC)
                    kt.append(_ld(kb, pl.ds(g * RB + 8 * c, 8), t0 + n, zs[-1 - LAG] if (i // 4) % P == 0 else None))
                mx = [_dot(qbd, jnp.concatenate(kt[n * MC:(n + 1) * MC], axis=0)) for n in range(TC)]
                for n, t in enumerate(ts):
                    a5, a6, a7 = acc[n][5], acc[n][6], acc[n][7]
                    z = jnp.where(odd, a7, a6) + pltpu.roll(jnp.where(odd, a6, a7), 1, 0)
                    z5 = a5 + pltpu.roll(a5, 1, 0)
                    u = jnp.where(bit1, z, z5) + pltpu.roll(jnp.where(bit1, z5, z), 2, 0)
                    r = u + pltpu.roll(u, 4, 0)
                    s_ref[g, :, t * 128:(t + 1) * 128] = mx[n] + jnp.where(sub >= 5, r, 0.0)

        for g in range(NG):
            s = s_ref[g] * (DH ** -0.5)
            e = jnp.exp(s - jnp.max(s, axis=-1, keepdims=True))
            s_ref[g] = e
            l_ref[g] = jnp.broadcast_to(jnp.sum(e, axis=-1, keepdims=True), (G, 128))

        @pl.when(first)
        def _():
            @pl.loop(0, NG)
            def _(g):
                for c in v_cp(g):
                    c.wait()

                def xpose(c, carry):
                    rows = pl.ds(g * RB + 8 * c, 8)
                    for t in range(NT):
                        tt = pltpu.bitcast(_ld(vb, rows, t).T, jnp.uint32)
                        vb.bitcast(jnp.uint32)[rows, t] = tt.reshape(8, 8, 128)
                    return carry
                lax.fori_loop(0, MC, xpose, 0)

        zs = [zero] * LAG
        for g in range(NG):
            p = s_ref[g].astype(BF)
            inv = 1.0 / l_ref[g]
            vu = vb.bitcast(jnp.uint32)
            nb = VB // MC
            for c in range(MC):
                rows = pl.ds(g * RB + 8 * c, 8)
                i0 = MB + c * nb
                h = i0 // (DH // 16)
                acc = [None] * (2 * nb)
                vt = []
                for t in range(NT):
                    pt = jnp.broadcast_to(s_ref[g, h:h + 1, t * 128:(t + 1) * 128], (8, 128))
                    for j in range(nb):
                        for e, w in enumerate(_unpack(vu[g * RB + i0 + j, t])):
                            acc[2 * j + e] = w * pt if t == 0 else acc[2 * j + e] + w * pt
                    zs.append(_tie(zs[-1], acc[t % (2 * nb)]))
                    vt.append(_ld(vb, rows, t, zs[-1 - LAG] if (t // 4) % P == 0 else None))
                sl = slice(c * 128, (c + 1) * 128)
                a_ref[g, :, sl] = jnp.where(diag[:, sl], _dot(p, jnp.concatenate(vt, axis=0)) * inv, 0.0)
                for j in range(nb):
                    for e in range(2):
                        acc_ref[g, pl.ds((c * nb + j) * 16 + e, 8, stride=2), :] = acc[2 * j + e]
            for c in range(MC, GR // 128):
                o = jnp.sum(acc_ref[g, (c - MC) * 128:(c - MC + 1) * 128].T, axis=0, keepdims=True)
                sl = slice(c * 128, (c + 1) * 128)
                a_ref[g, :, sl] = jnp.where(diag[:, sl], o * inv, 0.0)

        wait_first(first, wo_cp)
        a = jnp.concatenate([a_ref[g].astype(BF) for g in range(NG)], axis=1)
        y = jnp.concatenate([_dot(a, _ld(wob, slice(None), c)) for c in range(D // 128)], axis=1)
        x = x + jnp.sum(y, axis=0, keepdims=True)

        xn = _layernorm(x).astype(BF)
        wait_first(first, w1_cp)
        h = jnp.concatenate([_dot(xn, _ld(w1b, slice(None), c)) for c in range(F // 128)], axis=1)
        h = jax.nn.gelu(h + b1, approximate=True).astype(BF)
        wait_first(first, w2_cp)
        y = jnp.concatenate([_dot(h, _ld(w2b, slice(None), c)) for c in range(D // 128)], axis=1)
        return x + (y + b2)

    for c in small:
        c.wait()
    b1 = b1_ref[...].astype(F32).reshape(1, F)
    b2 = b2_ref[...].astype(F32).reshape(1, D)
    x0 = jnp.broadcast_to(x_ref[0].astype(F32), (8, D))
    x = lax.fori_loop(0, 2, layer, x0)
    o_ref[0] = x[0:1].astype(o_ref.dtype)


@jax.jit
def pallas_interleave_layers__sliding_block_cached__dense_activation_gelu__decode_kernel(
    A_x: jax.Array,
    A_k_cache: jax.Array,
    A_v_cache: jax.Array,
    A_wq: jax.Array,
    A_wo: jax.Array,
    B_x: jax.Array,
    B_w1: jax.Array,
    B_b1: jax.Array,
    B_w2: jax.Array,
    B_b2: jax.Array,
):
    del B_x
    kt = _tiles_view(jnp.swapaxes(A_k_cache, 2, 3).reshape(H * DH, SK))
    vt = _tiles_view(jnp.swapaxes(A_v_cache, 2, 3).reshape(H * DH, SK))
    vmem = pl.BlockSpec(memory_space=pltpu.VMEM)
    hbm = pl.BlockSpec(memory_space=pl.ANY)
    return pl.pallas_call(
        _kernel,
        out_shape=jax.ShapeDtypeStruct(A_x.shape, A_x.dtype),
        in_specs=[hbm] * 9,
        out_specs=vmem,
        scratch_shapes=[
            pltpu.VMEM((H * DH // 16, NT + 1, 16, 128), BF),
            pltpu.VMEM((H * DH // 16, NT + 1, 16, 128), BF),
            pltpu.VMEM((D // 16, H * DH // 128, 16, 128), BF),
            pltpu.VMEM((H * DH // 16, D // 128, 16, 128), BF),
            pltpu.VMEM((D // 16, F // 128, 16, 128), BF),
            pltpu.VMEM((F // 16, D // 128, 16, 128), BF),
            pltpu.VMEM((NG, G, MC * 128), F32),
            pltpu.VMEM((NG, G, W), F32),
            pltpu.VMEM((NG, G, 128), F32),
            pltpu.VMEM((NG, G, GR), F32),
            pltpu.VMEM((NG, 2, VB * 8, 128), F32),
            pltpu.VMEM((NG, VB * 16, 128), F32),
            pltpu.VMEM((1, 1, D), BF),
            pltpu.VMEM((F,), BF),
            pltpu.VMEM((D,), BF),
            pltpu.SemaphoreType.DMA((4 + 2 * NG, 2)),
            pltpu.SemaphoreType.DMA((3,)),
        ],
        compiler_params=pltpu.CompilerParams(vmem_limit_bytes=126 * 1024 * 1024),
    )(A_x, B_b1, B_b2, kt, vt,
      _tiles_view(A_wq), _tiles_view(A_wo), _tiles_view(B_w1), _tiles_view(B_w2))
```

```python
import jax
import jax.numpy as jnp
from jax import lax
import jax.experimental.pallas as pl
import jax.experimental.pallas.tpu as pltpu

H, DH, D, F = 32, 192, 640, 1536
SK, W = 32768, 4096
G = 8
NG = H // G
GR = G * DH
RB = GR // 16
NT = W // 128
MC = 8
MB = MC * 8
VB = RB - MB
TC = 4
P = 2
LAG = 4
EPS = 1e-5
BF, F32 = jnp.bfloat16, jnp.float32


def _tiles_view(a):
    r, c = a.shape
    return a.reshape(r // 16, 2, 8, c // 128, 128).transpose(0, 1, 3, 2, 4)


def _ld(buf, rows, col, zero=None):
    w = buf.bitcast(jnp.uint32)[rows, col]
    w = w.reshape(w.shape[0] * 8, 128)
    if zero is not None:
        w = jnp.concatenate([w[:-8], w[-8:] | zero], axis=0)
    return pltpu.bitcast(w, BF)


def _tie(zero, acc):
    return zero & pltpu.bitcast(acc, jnp.uint32)


def _unpack(w):
    return pltpu.bitcast(w << 16, F32), pltpu.bitcast(w & jnp.uint32(0xFFFF0000), F32)


def _dot(a, b):
    return jnp.dot(a, b, preferred_element_type=F32)


def _layernorm(x):
    m = jnp.sum(x, axis=-1, keepdims=True) * (1.0 / D)
    c = x - m
    v = jnp.sum(c * c, axis=-1, keepdims=True) * (1.0 / D)
    return c / jnp.sqrt(v + EPS)


def _kernel(x_hbm, b1_hbm, b2_hbm, k_hbm, v_hbm, wq_hbm, wo_hbm, w1_hbm, w2_hbm,
            o_ref, kb, vb, wqb, wob, w1b, w2b, q_ref, s_ref, l_ref, a_ref,
            qm_ref, acc_ref, x_ref, b1_ref, b2_ref, sems, small_sems):
    def copies(src, dst, r0, c0, sem):
        nc = src.shape[2] - c0
        return [pltpu.make_async_copy(
            src.at[pl.ds(r0, dst.shape[0]), a, pl.ds(c0, nc)],
            dst.at[:, pl.ds(0, nc), pl.ds(8 * a, 8), :],
            sems.at[sem, a]) for a in range(2)]

    c0 = (SK - W) // 128
    wq_cp = copies(wq_hbm, wqb, 0, 0, 0)
    k_cp = copies(k_hbm, kb, 0, c0, 1)
    v_cps = [copies(v_hbm, vb[g], g * RB, c0, 2 + g) for g in range(NG)]
    wo_cp = copies(wo_hbm, wob, 0, 0, 2 + NG)
    w1_cp = copies(w1_hbm, w1b, 0, 0, 3 + NG)
    w2_cp = copies(w2_hbm, w2b, 0, 0, 4 + NG)
    small = [pltpu.make_async_copy(s, d, small_sems.at[i]) for i, (s, d) in enumerate(
        [(x_hbm, x_ref), (b1_hbm, b1_ref), (b2_hbm, b2_ref)])]
    stream = [wq_cp, small, k_cp, *v_cps, wo_cp, w1_cp, w2_cp]
    for cps in stream:
        for c in cps:
            c.start()

    def wait_first(first, cps):
        @pl.when(first)
        def _():
            for c in cps:
                c.wait()

    col = lax.broadcasted_iota(jnp.int32, (G, GR), 1)
    row = lax.broadcasted_iota(jnp.int32, (G, GR), 0)
    diag = (col >= row * DH) & (col < (row + 1) * DH)
    sub = lax.broadcasted_iota(jnp.int32, (8, 128), 0)
    odd = (sub & 1) != 0
    bit1 = (sub & 2) != 0

    def layer(it, x):
        first = it == 0
        zero = jnp.full((8, 128), it >> 1, jnp.int32).astype(jnp.uint32)

        xn = _layernorm(x).astype(BF)
        wait_first(first, wq_cp)
        nj = GR // 128
        ties = []
        for g in range(NG):
            for j in range(MC, nj):
                q = _dot(xn, _ld(wqb, slice(None), g * nj + j))
                qc = jnp.broadcast_to(q[0:1], (128, 128)).astype(BF).T
                for e, w in enumerate(_unpack(pltpu.bitcast(qc, jnp.uint32))):
                    qm_ref[g, (j - MC) * 8:(j - MC + 1) * 8, e] = w.reshape(8, 8, 128)
                ties.append(_tie(zero, w[56:64]))
        ties = [None] * 4 + ties
        for g in range(NG):
            for j in range(MC):
                z = ties.pop(0) if ties else None
                w = jnp.concatenate([_ld(wqb, pl.ds(8 * r, 8), g * nj + j, z) for r in range(D // 128)])
                sl = slice(j * 128, (j + 1) * 128)
                q_ref[g, :, sl] = jnp.where(diag[:, sl], _dot(xn, w), 0.0)

        wait_first(first, k_cp)
        zs = [zero] * LAG
        for g in range(NG):
            qbd = q_ref[g].astype(BF)
            ku = kb.bitcast(jnp.uint32)
            for t0 in range(0, NT, TC):
                ts = range(t0, t0 + TC)
                acc = [{} for _ in ts]
                kt = []
                for i in range(MB, RB):
                    qlo = qm_ref[g, i - MB, 0]
                    qhi = qm_ref[g, i - MB, 1]
                    h = i // (DH // 16)
                    for n, t in enumerate(ts):
                        lo, hi = _unpack(ku[g * RB + i, t])
                        part = acc[n][h] + lo * qlo if h in acc[n] else lo * qlo
                        acc[n][h] = part + hi * qhi
                    zs.append(_tie(zs[-1], acc[i % TC][h]))
                    n, c = divmod(i - MB, MC)
                    kt.append(_ld(kb, pl.ds(g * RB + 8 * c, 8), t0 + n, zs[-1 - LAG] if (i // 4) % P == 0 else None))
                mx = [_dot(qbd, jnp.concatenate(kt[n * MC:(n + 1) * MC], axis=0)) for n in range(TC)]
                for n, t in enumerate(ts):
                    a5, a6, a7 = acc[n][5], acc[n][6], acc[n][7]
                    z = jnp.where(odd, a7, a6) + pltpu.roll(jnp.where(odd, a6, a7), 1, 0)
                    z5 = a5 + pltpu.roll(a5, 1, 0)
                    u = jnp.where(bit1, z, z5) + pltpu.roll(jnp.where(bit1, z5, z), 2, 0)
                    r = u + pltpu.roll(u, 4, 0)
                    s_ref[g, :, t * 128:(t + 1) * 128] = mx[n] + jnp.where(sub >= 5, r, 0.0)

        def land_v(groups):
            @pl.when(first)
            def _():
                for g in groups:
                    for c in v_cps[g]:
                        c.wait()

                    @pl.loop(0, MC)
                    def _(c):
                        rows = pl.ds(8 * c, 8)
                        for t in range(NT):
                            vb[g][rows, t] = _ld(vb[g], rows, t).T.reshape(8, 16, 128)

        land_v(range(NG // 2))
        for g in range(NG):
            s = s_ref[g] * (DH ** -0.5)
            e = jnp.exp(s - jnp.max(s, axis=-1, keepdims=True))
            s_ref[g] = e
            l_ref[g] = jnp.broadcast_to(jnp.sum(e, axis=-1, keepdims=True), (G, 128))

        land_v(range(NG // 2, NG))

        zs = [zero] * LAG
        for g in range(NG):
            p = s_ref[g].astype(BF)
            inv = 1.0 / l_ref[g]
            vu = vb[g].bitcast(jnp.uint32)
            nb = VB // MC
            for c in range(MC):
                rows = pl.ds(8 * c, 8)
                i0 = MB + c * nb
                h = i0 // (DH // 16)
                acc = [None] * (2 * nb)
                vt = []
                for t in range(NT):
                    pt = jnp.broadcast_to(s_ref[g, h:h + 1, t * 128:(t + 1) * 128], (8, 128))
                    for j in range(nb):
                        for e, w in enumerate(_unpack(vu[i0 + j, t])):
                            acc[2 * j + e] = w * pt if t == 0 else acc[2 * j + e] + w * pt
                    zs.append(_tie(zs[-1], acc[t % (2 * nb)]))
                    vt.append(_ld(vb[g], rows, t, zs[-1 - LAG] if (t // 4) % P == 0 else None))
                sl = slice(c * 128, (c + 1) * 128)
                a_ref[g, :, sl] = jnp.where(diag[:, sl], _dot(p, jnp.concatenate(vt, axis=0)) * inv, 0.0)
                for j in range(nb):
                    for e in range(2):
                        acc_ref[g, pl.ds((c * nb + j) * 16 + e, 8, stride=2), :] = acc[2 * j + e]
            for c in range(MC, GR // 128):
                o = jnp.sum(acc_ref[g, (c - MC) * 128:(c - MC + 1) * 128].T, axis=0, keepdims=True)
                sl = slice(c * 128, (c + 1) * 128)
                a_ref[g, :, sl] = jnp.where(diag[:, sl], o * inv, 0.0)

        wait_first(first, wo_cp)
        a = jnp.concatenate([a_ref[g].astype(BF) for g in range(NG)], axis=1)
        y = jnp.concatenate([_dot(a, _ld(wob, slice(None), c)) for c in range(D // 128)], axis=1)
        x = x + jnp.sum(y, axis=0, keepdims=True)

        xn = _layernorm(x).astype(BF)
        wait_first(first, w1_cp)
        h = jnp.concatenate([_dot(xn, _ld(w1b, slice(None), c)) for c in range(F // 128)], axis=1)
        h = jax.nn.gelu(h + b1, approximate=True).astype(BF)
        wait_first(first, w2_cp)
        y = jnp.concatenate([_dot(h, _ld(w2b, slice(None), c)) for c in range(D // 128)], axis=1)
        return x + (y + b2)

    for c in small:
        c.wait()
    b1 = b1_ref[...].astype(F32).reshape(1, F)
    b2 = b2_ref[...].astype(F32).reshape(1, D)
    x0 = jnp.broadcast_to(x_ref[0].astype(F32), (8, D))
    x = lax.fori_loop(0, 2, layer, x0)
    o_ref[0] = x[0:1].astype(o_ref.dtype)


@jax.jit
def pallas_interleave_layers__sliding_block_cached__dense_activation_gelu__decode_kernel(
    A_x: jax.Array,
    A_k_cache: jax.Array,
    A_v_cache: jax.Array,
    A_wq: jax.Array,
    A_wo: jax.Array,
    B_x: jax.Array,
    B_w1: jax.Array,
    B_b1: jax.Array,
    B_w2: jax.Array,
    B_b2: jax.Array,
):
    del B_x
    kt = _tiles_view(jnp.swapaxes(A_k_cache, 2, 3).reshape(H * DH, SK))
    vt = _tiles_view(jnp.swapaxes(A_v_cache, 2, 3).reshape(H * DH, SK))
    vmem = pl.BlockSpec(memory_space=pltpu.VMEM)
    hbm = pl.BlockSpec(memory_space=pl.ANY)
    return pl.pallas_call(
        _kernel,
        out_shape=jax.ShapeDtypeStruct(A_x.shape, A_x.dtype),
        in_specs=[hbm] * 9,
        out_specs=vmem,
        scratch_shapes=[
            pltpu.VMEM((H * DH // 16, NT + 1, 16, 128), BF),
            [pltpu.VMEM((RB, NT + 1, 16, 128), BF)] * NG,
            pltpu.VMEM((D // 16, H * DH // 128, 16, 128), BF),
            pltpu.VMEM((H * DH // 16, D // 128, 16, 128), BF),
            pltpu.VMEM((D // 16, F // 128, 16, 128), BF),
            pltpu.VMEM((F // 16, D // 128, 16, 128), BF),
            pltpu.VMEM((NG, G, MC * 128), F32),
            pltpu.VMEM((NG, G, W), F32),
            pltpu.VMEM((NG, G, 128), F32),
            pltpu.VMEM((NG, G, GR), F32),
            pltpu.VMEM((NG, VB, 2, 8, 128), F32),
            pltpu.VMEM((NG, VB * 16, 128), F32),
            pltpu.VMEM((1, 1, D), BF),
            pltpu.VMEM((F,), BF),
            pltpu.VMEM((D,), BF),
            pltpu.SemaphoreType.DMA((5 + NG, 2)),
            pltpu.SemaphoreType.DMA((3,)),
        ],
        compiler_params=pltpu.CompilerParams(vmem_limit_bytes=126 * 1024 * 1024),
    )(A_x, B_b1, B_b2, kt, vt,
      _tiles_view(A_wq), _tiles_view(A_wo), _tiles_view(B_w1), _tiles_view(B_w2))
```

```python
import jax
import jax.numpy as jnp
import numpy as np
from jax import lax
import jax.experimental.pallas as pl
import jax.experimental.pallas.tpu as pltpu

H, DH, D, F = 32, 192, 640, 1536
SK, W = 32768, 4096
G = 8
NG = H // G
GR = G * DH
NJ = GR // 128
RB = GR // 16
HB = DH // 16
NT = W // 128
ND = D // 128
MC = 8
MB = MC * 8
VB = RB - MB
TC = 4
LAG, WLAG = 4, 12
F1 = 1280
EPS = 1e-5
BF, F32, U32 = jnp.bfloat16, jnp.float32, jnp.uint32


def _tiles_view(a):
    r, c = a.shape
    return a.reshape(r // 16, 2, 8, c // 128, 128).transpose(0, 1, 3, 2, 4)


def _ld(buf, rows, col, zero=None):
    w = buf.bitcast(U32)[rows, col]
    w = w.reshape(w.shape[0] * 8, 128)
    if zero is not None:
        w = jnp.concatenate([w[:-8], w[-8:] | zero], axis=0)
    return pltpu.bitcast(w, BF)


def _tie(zero, acc):
    return zero & pltpu.bitcast(acc, U32)


def _unpack(w):
    return pltpu.bitcast(w << 16, F32), pltpu.bitcast(w & np.uint32(0xFFFF0000), F32)


def _dot(a, b):
    return jnp.dot(a, b, preferred_element_type=F32)


def _matvec(a, buf):
    return jnp.concatenate([_dot(a, _ld(buf, slice(None), c)) for c in range(buf.shape[1])], axis=1)


def _layernorm(x):
    m = jnp.sum(x, axis=-1, keepdims=True) * (1.0 / D)
    c = x - m
    v = jnp.sum(c * c, axis=-1, keepdims=True) * (1.0 / D)
    return c / jnp.sqrt(v + EPS)


def _kernel(x_hbm, b1_hbm, b2_hbm, k_hbm, v_hbm, wq_hbm, wo_hbm, w1_hbm, w2_hbm,
            o_ref, kb, vb, wqb, wob, w1b, w2b, q_ref, s_ref, l_ref, a_ref,
            qm_ref, am_ref, x_ref, b1_ref, b2_ref, sems, small_sems):
    def copies(src, dst, r0, c0, sem):
        nc = src.shape[2] - c0
        return [pltpu.make_async_copy(
            src.at[pl.ds(r0, dst.shape[0]), a, pl.ds(c0, nc)],
            dst.at[:, pl.ds(0, nc), pl.ds(8 * a, 8), :],
            sems.at[sem, a]) for a in range(2)]

    c0 = (SK - W) // 128
    wq_cp = copies(wq_hbm, wqb, 0, 0, 0)
    k_cp = copies(k_hbm, kb, 0, c0, 1)
    v_cps = [copies(v_hbm, vb[g], g * RB, c0, 2 + g) for g in range(NG)]
    wo_cp = copies(wo_hbm, wob, 0, 0, 2 + NG)
    w1_cp = copies(w1_hbm, w1b, 0, 0, 3 + NG)
    w2_cps = [copies(w2_hbm, w2b[0], 0, 0, 4 + NG), copies(w2_hbm, w2b[1], F1 // 16, 0, 5 + NG)]
    small = [pltpu.make_async_copy(s, d, small_sems.at[i]) for i, (s, d) in enumerate(
        [(x_hbm, x_ref), (b1_hbm, b1_ref), (b2_hbm, b2_ref)])]
    for cps in [wq_cp, small, k_cp, *v_cps, wo_cp, w1_cp, *w2_cps]:
        for c in cps:
            c.start()

    def wait_first(first, cps):
        @pl.when(first)
        def _():
            for c in cps:
                c.wait()

    col = lax.broadcasted_iota(jnp.int32, (G, GR), 1)
    row = lax.broadcasted_iota(jnp.int32, (G, GR), 0)
    diag = (col >= row * DH) & (col < (row + 1) * DH)
    sub = lax.broadcasted_iota(jnp.int32, (8, 128), 0)
    odd = (sub & 1) != 0
    bit1 = (sub & 2) != 0

    def layer(it, x):
        first = it == 0
        zero = jnp.full((8, 128), it >> 1, jnp.int32).astype(U32)

        xn = _layernorm(x).astype(BF)
        wait_first(first, wq_cp)
        ties = [None] * 4
        for g in range(NG):
            for j in range(MC, NJ):
                q = _dot(xn, _ld(wqb, slice(None), g * NJ + j))
                qc = jnp.broadcast_to(q[0:1], (128, 128)).astype(BF).T
                for e, w in enumerate(_unpack(pltpu.bitcast(qc, U32))):
                    qm_ref[g, (j - MC) * 8:(j - MC + 1) * 8, e] = w.reshape(8, 8, 128)
                ties.append(_tie(zero, w[56:64]))
        for g in range(NG):
            for j in range(MC):
                z = ties.pop(0) if ties else None
                w = jnp.concatenate([_ld(wqb, pl.ds(8 * r, 8), g * NJ + j, z) for r in range(ND)])
                sl = slice(j * 128, (j + 1) * 128)
                q_ref[g, :, sl] = jnp.where(diag[:, sl], _dot(xn, w), 0.0)

        wait_first(first, k_cp)
        ku = kb.bitcast(U32)
        zs = [zero] * LAG
        for g in range(NG):
            qbd = q_ref[g].astype(BF)
            for t0 in range(0, NT, TC):
                acc = [{} for _ in range(TC)]
                kt = []
                for i in range(MB, RB):
                    qlo, qhi = qm_ref[g, i - MB, 0], qm_ref[g, i - MB, 1]
                    h = i // HB
                    for n in range(TC):
                        lo, hi = _unpack(ku[g * RB + i, t0 + n])
                        part = acc[n][h] + lo * qlo if h in acc[n] else lo * qlo
                        acc[n][h] = part + hi * qhi
                    zs.append(_tie(zs[-1], acc[i % TC][h]))
                    n, c = divmod(i - MB, MC)
                    z = zs[-1 - LAG] if i % 8 < 4 else None
                    kt.append(_ld(kb, pl.ds(g * RB + 8 * c, 8), t0 + n, z))
                mx = [_dot(qbd, jnp.concatenate(kt[n * MC:(n + 1) * MC])) for n in range(TC)]
                for n in range(TC):
                    a5, a6, a7 = acc[n][5], acc[n][6], acc[n][7]
                    z67 = jnp.where(odd, a7, a6) + pltpu.roll(jnp.where(odd, a6, a7), 1, 0)
                    z5 = a5 + pltpu.roll(a5, 1, 0)
                    u = jnp.where(bit1, z67, z5) + pltpu.roll(jnp.where(bit1, z5, z67), 2, 0)
                    r = u + pltpu.roll(u, 4, 0)
                    sl = slice((t0 + n) * 128, (t0 + n + 1) * 128)
                    s_ref[g, :, sl] = mx[n] + jnp.where(sub >= 5, r, 0.0)

        def land_v(groups):
            @pl.when(first)
            def _():
                for g in groups:
                    for c in v_cps[g]:
                        c.wait()

                    @pl.loop(0, MC)
                    def _(c):
                        rows = pl.ds(8 * c, 8)
                        for t in range(NT):
                            vb[g][rows, t] = _ld(vb[g], rows, t).T.reshape(8, 16, 128)

        land_v(range(NG // 2))
        for g in range(NG):
            s = s_ref[g] * (DH ** -0.5)
            e = jnp.exp(s - jnp.max(s, axis=-1, keepdims=True))
            s_ref[g] = e
            l_ref[g] = jnp.broadcast_to(jnp.sum(e, axis=-1, keepdims=True), (G, 128))
        land_v(range(NG // 2, NG))

        nb = VB // MC
        zs = [zero] * LAG
        for g in range(NG):
            p = s_ref[g].astype(BF)
            inv = 1.0 / l_ref[g]
            vu = vb[g].bitcast(U32)
            for c in range(MC):
                i0 = MB + c * nb
                h = i0 // HB
                acc = [None] * (2 * nb)
                vt = []
                for t in range(NT):
                    pt = jnp.broadcast_to(s_ref[g, h:h + 1, t * 128:(t + 1) * 128], (8, 128))
                    for j in range(nb):
                        for e, w in enumerate(_unpack(vu[i0 + j, t])):
                            acc[2 * j + e] = w * pt if t == 0 else acc[2 * j + e] + w * pt
                    zs.append(_tie(zs[-1], acc[t % (2 * nb)]))
                    vt.append(_ld(vb[g], pl.ds(8 * c, 8), t, zs[-1 - LAG] if t % 8 < 4 else None))
                sl = slice(c * 128, (c + 1) * 128)
                a_ref[g, :, sl] = jnp.where(diag[:, sl], _dot(p, jnp.concatenate(vt)) * inv, 0.0)
                for v in acc:
                    zs[-1] = _tie(zs[-1], v)
                inv_h = jnp.broadcast_to(inv[h:h + 1], (8, 128))
                for j in range(nb):
                    for e in range(2):
                        o = jnp.sum(acc[2 * j + e], axis=1, keepdims=True)
                        am_ref[g, c * nb + j, e] = o * inv_h

        wait_first(first, wo_cp)
        a = jnp.concatenate([a_ref[g].astype(BF) for g in range(NG)], axis=1)
        tiles = [(c, g * NJ + j) for c in range(ND) for g in range(NG) for j in range(MC)]
        wt, acc, zs = [], [None] * ND, [zero] * WLAG
        for g in range(NG):
            for i in range(VB):
                alo, ahi = am_ref[g, i, 0], am_ref[g, i, 1]
                for c in range(ND):
                    lo, hi = _unpack(wob.bitcast(U32)[g * RB + MB + i, c])
                    term = lo * alo + hi * ahi
                    acc[c] = term if acc[c] is None else acc[c] + term
                zs.append(_tie(zs[-1], acc[len(zs) % ND]))
                while len(wt) * NG * VB < (len(zs) - WLAG) * len(tiles):
                    c, r = tiles[len(wt)]
                    z = zs[-1 - WLAG] if len(wt) % 8 < 4 else None
                    wt.append(_ld(wob, pl.ds(8 * r, 8), c, z))
        n = NG * MC
        y = jnp.concatenate(
            [_dot(a, jnp.concatenate(wt[c * n:(c + 1) * n])) + acc[c] for c in range(ND)], axis=1)
        x = x + jnp.sum(y, axis=0, keepdims=True)

        xn = _layernorm(x).astype(BF)
        wait_first(first, w1_cp)
        hid = jax.nn.gelu(_matvec(xn, w1b) + b1, approximate=True).astype(BF)
        y = b2
        for cps, w2, part in zip(w2_cps, w2b, (hid[:, :F1], hid[:, F1:])):
            wait_first(first, cps)
            y = y + _matvec(part, w2)
        return x + y

    for c in small:
        c.wait()
    b1 = b1_ref[...].astype(F32).reshape(1, F)
    b2 = b2_ref[...].astype(F32).reshape(1, D)
    x0 = jnp.broadcast_to(x_ref[0].astype(F32), (8, D))
    x = lax.fori_loop(0, 2, layer, x0)
    o_ref[0] = x[0:1].astype(o_ref.dtype)


@jax.jit
def pallas_interleave_layers__sliding_block_cached__dense_activation_gelu__decode_kernel(
    A_x: jax.Array,
    A_k_cache: jax.Array,
    A_v_cache: jax.Array,
    A_wq: jax.Array,
    A_wo: jax.Array,
    B_x: jax.Array,
    B_w1: jax.Array,
    B_b1: jax.Array,
    B_w2: jax.Array,
    B_b2: jax.Array,
):
    del B_x
    kt = _tiles_view(jnp.swapaxes(A_k_cache, 2, 3).reshape(H * DH, SK))
    vt = _tiles_view(jnp.swapaxes(A_v_cache, 2, 3).reshape(H * DH, SK))
    return pl.pallas_call(
        _kernel,
        out_shape=jax.ShapeDtypeStruct(A_x.shape, A_x.dtype),
        in_specs=[pl.BlockSpec(memory_space=pl.ANY)] * 9,
        out_specs=pl.BlockSpec(memory_space=pltpu.VMEM),
        scratch_shapes=[
            pltpu.VMEM((NG * RB, NT + 1, 16, 128), BF),
            [pltpu.VMEM((RB, NT + 1, 16, 128), BF)] * NG,
            pltpu.VMEM((D // 16, NG * NJ, 16, 128), BF),
            pltpu.VMEM((NG * RB, ND, 16, 128), BF),
            pltpu.VMEM((D // 16, F // 128, 16, 128), BF),
            [pltpu.VMEM((n // 16, ND, 16, 128), BF) for n in (F1, F - F1)],
            pltpu.VMEM((NG, G, MC * 128), F32),
            pltpu.VMEM((NG, G, W), F32),
            pltpu.VMEM((NG, G, 128), F32),
            pltpu.VMEM((NG, G, MC * 128), F32),
            pltpu.VMEM((NG, VB, 2, 8, 128), F32),
            pltpu.VMEM((NG, VB, 2, 8, 128), F32),
            pltpu.VMEM((1, 1, D), BF),
            pltpu.VMEM((F,), BF),
            pltpu.VMEM((D,), BF),
            pltpu.SemaphoreType.DMA((6 + NG, 2)),
            pltpu.SemaphoreType.DMA((3,)),
        ],
        compiler_params=pltpu.CompilerParams(vmem_limit_bytes=126 * 1024 * 1024),
    )(A_x, B_b1, B_b2, kt, vt,
      _tiles_view(A_wq), _tiles_view(A_wo), _tiles_view(B_w1), _tiles_view(B_w2))
```
